```python
import jax
import jax.numpy as jnp

def _softmax(x, axis=-1):
    return jax.nn.softmax(x, axis=axis)
def _gelu(x):
    return jax.nn.gelu(x, approximate=True)
def _silu(x):
    return jax.nn.silu(x)
def _sigmoid(x):
    return jax.nn.sigmoid(x)
def _layernorm(x, axis=-1, eps=1e-5):
    m = jnp.mean(x, axis=axis, keepdims=True)
    v = jnp.var(x, axis=axis, keepdims=True)
    return (x - m) / jnp.sqrt(v + eps)
def _scatter_add(tgt, idx, src, axis=0):
    return tgt.at[idx].add(src)
def _segment_sum(src, seg, n):
    return jax.ops.segment_sum(src, seg, n)
class _Rng:
    def __init__(self, key):
        self._k = key
    def _next(self):
        self._k, sub = jax.random.split(self._k)
        return sub
    def normal(self, shape):
        return jax.random.normal(self._next(), shape, dtype=jnp.bfloat16)
    def randint(self, lo, hi, shape):
        return jax.random.randint(self._next(), shape, lo, hi, dtype=jnp.int32)
    def uniform(self, shape, lo=0.0, hi=1.0):
        return jax.random.uniform(self._next(), shape, jnp.bfloat16, lo, hi)
    def permutation(self, n):
        return jax.random.permutation(self._next(), n)


kernel_name = 'recurrent_scan__sliding_block_cached__glu_gated_swiglu__decode'

def setup_inputs():
    _rng = _Rng(jax.random.key(int.from_bytes(__import__("os").urandom(4), "little")))
    _w = (lambda a: (lambda t: t.astype(jnp.bfloat16) if jnp.issubdtype(t.dtype, jnp.floating) else t)(jnp.asarray(a)))
    def _A_setup():
        B, Sq, D = 1, 1, 640
        Hq, Hkv, Sk, Dh = 32, 32, 32768, 192
        assert Hq % Hkv == 0, (Hq, Hkv)
        return {
            "x": _w((lambda *s: _rng.normal(s) * 0.05)(B, Sq, D)),
            "k_cache": _w((lambda *s: _rng.normal(s) * 0.05)(B, Hkv, Sk, Dh)),
            "v_cache": _w((lambda *s: _rng.normal(s) * 0.05)(B, Hkv, Sk, Dh)),
            "wq": _w((lambda *s: _rng.normal(s) * 0.05)(D, Hq * Dh) * (D ** -0.5)),
            "wo": _w((lambda *s: _rng.normal(s) * 0.05)(Hq * Dh, D) * ((Hq * Dh) ** -0.5)),
        }
    _A_in = _A_setup()

    def _B_setup():
        B, S, D, F = 1, 1, 640, 1536
        return {
            "x": _w((lambda *s: _rng.normal(s) * 0.05)(B, S, D)),
            "w1": _w((lambda *s: _rng.normal(s) * 0.05)(D, F) * (2.0 / D) ** 0.5),
            "w3": _w((lambda *s: _rng.normal(s) * 0.05)(D, F) * (2.0 / D) ** 0.5),
            "w2": _w((lambda *s: _rng.normal(s) * 0.05)(F, D) * (2.0 / F) ** 0.5),
        }
    _B_in = _B_setup()

    return {
        "A_x": _A_in["x"],
        "A_k_cache": _A_in["k_cache"],
        "A_v_cache": _A_in["v_cache"],
        "A_wq": _A_in["wq"],
        "A_wo": _A_in["wo"],
        "B_x": _B_in["x"],
        "B_w1": _B_in["w1"],
        "B_w3": _B_in["w3"],
        "B_w2": _B_in["w2"],
    }

def reference(A_x, A_k_cache, A_v_cache, A_wq, A_wo, B_x, B_w1, B_w3, B_w2):
    def _A_ref(x, k_cache, v_cache, wq, wo):
        B, Sq, D = x.shape
        Hq, Dh = 32, 192
        Hkv, Sk = k_cache.shape[1], k_cache.shape[2]
        W = min(4096, max(256, Sk // 4))
        rep = Hq // Hkv
        q = (lambda x, *d: x.transpose(*d))((x @ wq).reshape(B, Sq, Hq, Dh), 0, 2, 1, 3)
        k = jnp.repeat(k_cache[:, :, Sk - W:, :], rep, axis=1)
        v = jnp.repeat(v_cache[:, :, Sk - W:, :], rep, axis=1)
        scores = jnp.einsum("bhqd,bhkd->bhqk", q, k) * (Dh ** -0.5)
        p = _softmax(scores, axis=-1)
        o = jnp.einsum("bhqk,bhkd->bhqd", p, v)
        return (lambda x, *d: x.transpose(*d))(o, 0, 2, 1, 3).reshape(B, Sq, Hq * Dh) @ wo

    def _B_ref(x, w1, w3, w2):
        gate = jnp.einsum("bsd,df->bsf", x, w1)
        up = jnp.einsum("bsd,df->bsf", x, w3)
        h = _silu(gate) * up
        out = jnp.einsum("bsf,fd->bsd", h, w2)
        return out

    x = A_x
    xn = _layernorm(x, axis=-1)
    s = _A_ref(xn, A_k_cache, A_v_cache, A_wq, A_wo)
    g = _silu(_B_ref(xn, B_w1, B_w3, B_w2))
    return x + s * g
```

```python
import functools
import jax
import jax.numpy as jnp
from jax import lax
from jax.experimental import pallas as pl
from jax.experimental.pallas import tpu as pltpu

D, F, H, DH, SK = 640, 1536, 32, 192, 32768
W = min(4096, max(256, SK // 4))
NC = W // 128
HD = H * DH
f32, bf16 = jnp.float32, jnp.bfloat16


def _tree_sum(xs):
    xs = list(xs)
    while len(xs) > 1:
        xs = [xs[i] + xs[i + 1] if i + 1 < len(xs) else xs[i] for i in range(0, len(xs), 2)]
    return xs[0]


def _is_int(i):
    return isinstance(i, int)


def _shr(i, s):
    return i >> s if _is_int(i) else lax.shift_right_logical(i, s)


def _and(i, m):
    return i & m if _is_int(i) else lax.bitwise_and(i, m)


def _mo(i, m):
    return i if _is_int(i) else pl.multiple_of(i, m)


def make(KD=64, KR=128, VR=64, B1=99, WL=6, QT0=96):
    NQ, N1, N2, NO = 80, 40, 24, 192
    A = NQ + N1 + N2
    NKV = H * NC
    B0 = NO - B1
    T1 = [('wqL', NQ), ('w1', N1), ('w2a', N2), ('K', NKV), ('woa', B1)]
    T0 = [('wqR', NQ), ('w3', N1), ('w2b', N2), ('V', NKV), ('wob', B0)]
    NT = A + NKV + B1

    def locate(lst, t):
        for kind, n in lst:
            if 0 <= t < n:
                return kind, t
            t -= n
        return None, None

    def offset(lst, kind):
        o = 0
        for k, n in lst:
            if k == kind:
                return o
            o += n

    def _kernel(x_hbm, k_hbm, v_hbm, wq_hbm, wo_hbm, w1_hbm, w3_hbm, w2_hbm, o_ref,
                x_v, wq_v, wo_v, w1_v, w3_v, w2_v, kbuf, vbuf, qbc, obc, s_scr, p_scr, acc_ref, xn_s, g_s,
                sem_x, sem_w, sem_k, sem_v, sem_oa, sem_ob):
        WSEM = {'wqL': 0, 'wqR': 1, 'w1': 2, 'w3': 3, 'w2a': 4, 'w2b': 5}

        def cp(kind, i):
            if kind in ('wqL', 'wqR'):
                r0 = _mo(_shr(i, 1) * 16, 16)
                c0 = _mo(_and(i, 1) * 1536 + (0 if kind == 'wqL' else 3072), 128)
                sl = (pl.ds(r0, 16), pl.ds(c0, 1536))
                return pltpu.make_async_copy(wq_hbm.at[sl], wq_v.at[sl], sem_w.at[WSEM[kind]])
            if kind in ('w1', 'w3'):
                src, dst = (w1_hbm, w1_v) if kind == 'w1' else (w3_hbm, w3_v)
                sl = pl.ds(_mo(i * 16, 16), 16)
                return pltpu.make_async_copy(src.at[sl], dst.at[sl], sem_w.at[WSEM[kind]])
            if kind in ('w2a', 'w2b'):
                sl = pl.ds(_mo((i + (0 if kind == 'w2a' else N2)) * 32, 32), 32)
                return pltpu.make_async_copy(w2_hbm.at[sl], w2_v.at[sl], sem_w.at[WSEM[kind]])
            if kind in ('K', 'V'):
                src, buf, sem, ring = (k_hbm, kbuf, sem_k, KR) if kind == 'K' else (v_hbm, vbuf, sem_v, VR)
                r0 = _mo(_shr(i, 5) * DH, 8)
                c0 = _mo(SK - W + _and(i, NC - 1) * 128, 128)
                slot = _and(i, ring - 1)
                return pltpu.make_async_copy(src.at[pl.ds(r0, DH), pl.ds(c0, 128)], buf.at[slot], sem.at[slot])
            if kind in ('woa', 'wob'):
                u = i + (0 if kind == 'woa' else B1)
                sl = pl.ds(_mo(u * 32, 32), 32)
                sem = sem_oa.at[_and(i, 127)] if kind == 'woa' else sem_ob.at[_and(i, 15)]
                return pltpu.make_async_copy(wo_hbm.at[sl], wo_v.at[sl], sem)
            raise ValueError(kind)

        def wait_all(kind, n):
            if kind in ('wqR',):
                sl = (slice(None), pl.ds(3072, 3072))
                pltpu.make_async_copy(wq_v.at[sl], wq_v.at[sl], sem_w.at[WSEM[kind]]).wait()
            elif kind == 'w3':
                pltpu.make_async_copy(w3_v, w3_v, sem_w.at[WSEM[kind]]).wait()
            elif kind == 'w2b':
                sl = pl.ds(N2 * 32, N2 * 32)
                pltpu.make_async_copy(w2_v.at[sl], w2_v.at[sl], sem_w.at[WSEM[kind]]).wait()

        def starts(t, k1, o1, k0, o0):
            if k1 is not None:
                cp(k1, t + KD - o1).start(priority=1)
            if k0 is not None:
                cp(k0, t - o0).start(priority=0)

        x_cp = pltpu.make_async_copy(x_hbm, x_v, sem_x.at[0])
        for t in range(KD):
            k, i = locate(T1, t)
            cp(k, i).start(priority=1)
            if t == 0:
                x_cp.start(priority=0)

        def q_piece(j):
            c0 = _mo(j * 384, 128)
            q = jnp.dot(xn_s[...], wq_v[:, pl.ds(c0, 384)], preferred_element_type=f32)
            qb = q[0:1].astype(bf16)
            eye = (lax.broadcasted_iota(jnp.int32, (128, 128), 0) == lax.broadcasted_iota(jnp.int32, (128, 128), 1)).astype(bf16)
            for i in range(3):
                r = jnp.broadcast_to(qb[:, i * 128:(i + 1) * 128], (128, 128))
                qbc[pl.ds(_mo(j * 384 + i * 128, 128), 128), :] = lax.dot_general(
                    eye, r, (((1,), (1,)), ((), ())), preferred_element_type=f32)

        def qk(n, b, c):
            slot = _and(n, KR - 1)
            r0 = _mo(b * DH, 8)
            parts = []
            for g in range(DH // 16):
                k = kbuf[slot, pl.ds(g * 16, 16), :].astype(f32)
                parts.append(k * qbc[pl.ds(r0 + g * 16, 16), :])
            tt = _tree_sum(parts)
            s_scr[pl.ds(_mo(c * 8, 8), 8), :] = tt[0:8] + tt[8:16]

        def pv(n, c):
            slot = _and(n, VR - 1)
            p = jnp.broadcast_to(p_scr[pl.ds(c, 1), :], (16, 128))
            for g in range(DH // 16):
                v = vbuf[slot, pl.ds(g * 16, 16), :].astype(f32)
                acc_ref[pl.ds(g * 16, 16), :] += v * p

        def softmax():
            rows = [_tree_sum([s_scr[pl.ds(g * 64 + j, 8, stride=8), :] for j in range(8)]) for g in range(NC // 8)]
            s = jnp.concatenate(rows, axis=0) * (DH ** -0.5)
            m = jnp.max(jnp.max(s, axis=0, keepdims=True), axis=1, keepdims=True)
            p = jnp.exp(s - m)
            l = jnp.sum(jnp.sum(p, axis=0, keepdims=True), axis=1, keepdims=True)
            p_scr[...] = p
            return l

        def finalize(h, l):
            o = jnp.sum(acc_ref[...], axis=1, keepdims=True) / l
            obc[pl.ds(_mo(h * DH, 8), DH), :] = jnp.broadcast_to(o, (DH, 128))

        def wo_piece(u, y):
            r0 = _mo(u * 32, 32)
            for g in range(2):
                w = wo_v[pl.ds(r0 + g * 16, 16), :].astype(f32)
                ob = obc[pl.ds(r0 + g * 16, 16), :]
                pr = w * jnp.concatenate([ob] * (D // 128), axis=1)
                y = y + pr[0:8] + pr[8:16]
            return y

        def ffn():
            xn8 = xn_s[...]
            gate = jnp.dot(xn8, w1_v[...], preferred_element_type=f32)
            up = jnp.dot(xn8, w3_v[...], preferred_element_type=f32)
            hh = (gate * jax.nn.sigmoid(gate) * up).astype(bf16)
            ff = jnp.dot(hh, w2_v[...], preferred_element_type=f32)
            g_s[...] = ff * jax.nn.sigmoid(ff)

        x_cp.wait()
        x = x_v[...].reshape(1, D).astype(f32)
        mu = jnp.mean(x, axis=-1, keepdims=True)
        xc = x - mu
        var = jnp.mean(xc * xc, axis=-1, keepdims=True)
        xn_s[...] = jnp.broadcast_to((xc / jnp.sqrt(var + 1e-5)).astype(bf16), (8, D))

        cuts = {0, A, NQ, NQ + N1, QT0, QT0 + 16}
        o = 0
        for k, n in T1:
            o += n
            if 0 < o - KD < A:
                cuts.add(o - KD)
        cuts = sorted(c for c in cuts if 0 <= c <= A)
        for t0, t1 in zip(cuts[:-1], cuts[1:]):
            kw, _ = locate(T1, t0)
            k1, _ = locate(T1, t0 + KD)
            k0, _ = locate(T0, t0)
            if t0 == QT0:
                wait_all('wqR', NQ)

            def body(t, carry, kw=kw, k1=k1, k0=k0, t0=t0):
                cp(kw, t - offset(T1, kw)).wait()
                if t0 == QT0:
                    q_piece(t - QT0)
                starts(t, k1, offset(T1, k1), k0, offset(T0, k0))
                return carry
            lax.fori_loop(t0, t1, body, 0)

        oK, oV, oA, oB = offset(T1, 'K'), offset(T0, 'V'), offset(T1, 'woa'), offset(T0, 'wob')

        def block(b, do_pv, k1, l_prev):
            if do_pv:
                acc_ref[...] = jnp.zeros_like(acc_ref)

            def body(c, carry):
                n = b * NC + c
                cp('K', n).wait()
                if do_pv:
                    cp('V', n - NC).wait()
                qk(n, b, c)
                if do_pv:
                    pv(n - NC, c)
                starts(A + n, k1, offset(T1, k1), 'V', oV)
                return carry
            lax.fori_loop(0, NC, body, 0)
            if do_pv:
                finalize(b - 1, l_prev)
            return softmax()

        nl = KD // NC
        l = block(0, False, 'K', None)
        wait_all('w3', N1)
        wait_all('w2b', N2)
        ffn()
        l = lax.fori_loop(1, H - nl, lambda b, l: block(b, True, 'K', l), l)
        for b in range(H - nl, H):
            l = block(b, True, 'woa', l)

        acc_ref[...] = jnp.zeros_like(acc_ref)
        tB = A + NKV
        cuts = sorted({0, WL, NC, B1 - KD, B0, B0 + WL, B1})
        cuts = [c for c in cuts if 0 <= c <= B1]
        y = jnp.zeros((8, D), f32)
        for j0, j1 in zip(cuts[:-1], cuts[1:]):
            do_pv = j1 <= NC
            s1 = 'woa' if j0 + KD < B1 else None
            s0 = 'wob' if j0 < B0 else None
            w0 = WL <= j0 < B0 + WL

            def body(j, y, do_pv=do_pv, s1=s1, s0=s0, w0=w0):
                cp('woa', j).wait()
                if do_pv:
                    cp('V', NKV - NC + j).wait()
                if w0:
                    cp('wob', j - WL).wait()
                if do_pv:
                    pv(NKV - NC + j, j)
                y = wo_piece(j, y)
                if w0:
                    y = wo_piece(B1 + j - WL, y)
                starts(tB + j, s1, offset(T1, 'woa'), s0, offset(T0, 'wob'))
                return y
            y = lax.fori_loop(j0, j1, body, y)
            if j1 == NC:
                finalize(H - 1, l)

        s = jnp.sum(y, axis=0, keepdims=True)
        out = x_v[...].reshape(1, D).astype(f32) + s * g_s[0:1]
        o_ref[...] = out.astype(bf16).reshape(1, 1, D)

    def simulate():
        started, waited = set(), set()
        def st(k, i):
            n = dict(T1 + T0)[k]
            assert 0 <= i < n, (k, i)
            assert (k, i) not in started
            started.add((k, i))
        def wt(k, i):
            assert (k, i) in started, ('wait before start', k, i)
            assert (k, i) not in waited
            waited.add((k, i))
        for t in range(KD):
            st(*locate(T1, t))
        for t in range(NT):
            k, i = locate(T1, t)
            wt(k, i)
            if k == 'K' and i >= NC:
                wt('V', i - NC)
            if k == 'woa':
                if i < NC:
                    wt('V', NKV - NC + i)
                if WL <= i < B0 + WL:
                    wt('wob', i - WL)
            k1, i1 = locate(T1, t + KD)
            if k1 is not None:
                st(k1, i1)
            k0, i0 = locate(T0, t)
            if k0 is not None:
                st(k0, i0)
        for k in ('wqR', 'w3', 'w2b'):
            for i in range(dict(T0)[k]):
                wt(k, i)
        assert started == waited, (len(started), len(waited), sorted(started - waited)[:5])
        assert B0 + WL <= B1 and B1 <= 128 and WL < 16
        assert KD % NC == 0 and KD + 2 <= KR and VR >= NC + 2
        assert B1 <= 186 and (186 - B1) + WL >= NC
    simulate()

    @jax.jit
    def kernel_fn(A_x, A_k_cache, A_v_cache, A_wq, A_wo, B_x, B_w1, B_w3, B_w2):
        kT = jnp.swapaxes(A_k_cache, 2, 3).reshape(HD, SK)
        vT = jnp.swapaxes(A_v_cache, 2, 3).reshape(HD, SK)
        return pl.pallas_call(
            _kernel,
            in_specs=[pl.BlockSpec(memory_space=pl.ANY)] * 8,
            out_specs=pl.BlockSpec(memory_space=pltpu.VMEM),
            out_shape=jax.ShapeDtypeStruct((1, 1, D), bf16),
            scratch_shapes=[
                pltpu.VMEM((1, 1, D), bf16),
                pltpu.VMEM((D, HD), bf16),
                pltpu.VMEM((HD, D), bf16),
                pltpu.VMEM((D, F), bf16),
                pltpu.VMEM((D, F), bf16),
                pltpu.VMEM((F, D), bf16),
                pltpu.VMEM((KR, DH, 128), bf16),
                pltpu.VMEM((VR, DH, 128), bf16),
                pltpu.VMEM((HD, 128), f32),
                pltpu.VMEM((HD, 128), f32),
                pltpu.VMEM((NC * 8, 128), f32),
                pltpu.VMEM((NC, 128), f32),
                pltpu.VMEM((DH, 128), f32),
                pltpu.VMEM((8, D), bf16),
                pltpu.VMEM((8, D), f32),
                pltpu.SemaphoreType.DMA((1,)),
                pltpu.SemaphoreType.DMA((6,)),
                pltpu.SemaphoreType.DMA((KR,)),
                pltpu.SemaphoreType.DMA((VR,)),
                pltpu.SemaphoreType.DMA((128,)),
                pltpu.SemaphoreType.DMA((16,)),
            ],
            compiler_params=pltpu.CompilerParams(vmem_limit_bytes=100 * 1024 * 1024,
                                                 disable_bounds_checks=True, disable_semaphore_checks=True),
        )(A_x, kT, vT, A_wq, A_wo, B_w1, B_w3, B_w2)
    return kernel_fn

_impl = make()


@jax.jit
def pallas_recurrent_scan__sliding_block_cached__glu_gated_swiglu__decode_kernel(
        A_x, A_k_cache, A_v_cache, A_wq, A_wo, B_x, B_w1, B_w3, B_w2):
    return _impl(A_x, A_k_cache, A_v_cache, A_wq, A_wo, B_x, B_w1, B_w3, B_w2)
```

```python
import functools
import jax
import jax.numpy as jnp
from jax import lax
from jax.experimental import pallas as pl
from jax.experimental.pallas import tpu as pltpu

D, F, H, DH, SK = 640, 1536, 32, 192, 32768
W = min(4096, max(256, SK // 4))
NC = W // 128
HD = H * DH
f32, bf16 = jnp.float32, jnp.bfloat16


def _tree_sum(xs):
    xs = list(xs)
    while len(xs) > 1:
        xs = [xs[i] + xs[i + 1] if i + 1 < len(xs) else xs[i] for i in range(0, len(xs), 2)]
    return xs[0]


def _is_int(i):
    return isinstance(i, int)


def _shr(i, s):
    return i >> s if _is_int(i) else lax.shift_right_logical(i, s)


def _and(i, m):
    return i & m if _is_int(i) else lax.bitwise_and(i, m)


def _mo(i, m):
    return i if _is_int(i) else pl.multiple_of(i, m)


def make(KD=64, KR=128, VR=64, B1=99, WL=6, QT0=96, off=''):
    NQ, N1, N2, NO = 80, 40, 24, 192
    A = NQ + N1 + N2
    NKV = H * NC
    B0 = NO - B1
    T1 = [('wqL', NQ), ('w1', N1), ('w2a', N2), ('K', NKV), ('woa', B1)]
    T0 = [('wqR', NQ), ('w3', N1), ('w2b', N2), ('V', NKV), ('wob', B0)]
    NT = A + NKV + B1

    def locate(lst, t):
        for kind, n in lst:
            if 0 <= t < n:
                return kind, t
            t -= n
        return None, None

    def offset(lst, kind):
        o = 0
        for k, n in lst:
            if k == kind:
                return o
            o += n

    def _kernel(x_hbm, k_hbm, v_hbm, wq_hbm, wo_hbm, w1_hbm, w3_hbm, w2_hbm, o_ref,
                x_v, wq_v, wo_v, w1_v, w3_v, w2_v, kbuf, vbuf, qbc, qrow, obc, s_scr, p_scr, acc_ref, xn_s, g_s,
                sem_x, sem_w, sem_k, sem_v, sem_oa, sem_ob):
        WSEM = {'wqL': 0, 'wqR': 1, 'w1': 2, 'w3': 3, 'w2a': 4, 'w2b': 5}

        def cp(kind, i):
            if kind in ('wqL', 'wqR'):
                r0 = _mo(_shr(i, 1) * 16, 16)
                c0 = _mo(_and(i, 1) * 1536 + (0 if kind == 'wqL' else 3072), 128)
                sl = (pl.ds(r0, 16), pl.ds(c0, 1536))
                return pltpu.make_async_copy(wq_hbm.at[sl], wq_v.at[sl], sem_w.at[WSEM[kind]])
            if kind in ('w1', 'w3'):
                src, dst = (w1_hbm, w1_v) if kind == 'w1' else (w3_hbm, w3_v)
                sl = pl.ds(_mo(i * 16, 16), 16)
                return pltpu.make_async_copy(src.at[sl], dst.at[sl], sem_w.at[WSEM[kind]])
            if kind in ('w2a', 'w2b'):
                sl = pl.ds(_mo((i + (0 if kind == 'w2a' else N2)) * 32, 32), 32)
                return pltpu.make_async_copy(w2_hbm.at[sl], w2_v.at[sl], sem_w.at[WSEM[kind]])
            if kind in ('K', 'V'):
                src, buf, sem, ring = (k_hbm, kbuf, sem_k, KR) if kind == 'K' else (v_hbm, vbuf, sem_v, VR)
                r0 = _mo(_shr(i, 5) * DH, 8)
                c0 = _mo(SK - W + _and(i, NC - 1) * 128, 128)
                slot = _and(i, ring - 1)
                return pltpu.make_async_copy(src.at[pl.ds(r0, DH), pl.ds(c0, 128)], buf.at[slot], sem.at[slot])
            if kind in ('woa', 'wob'):
                u = i + (0 if kind == 'woa' else B1)
                sl = pl.ds(_mo(u * 32, 32), 32)
                sem = sem_oa.at[_and(i, 127)] if kind == 'woa' else sem_ob.at[_and(i, 15)]
                return pltpu.make_async_copy(wo_hbm.at[sl], wo_v.at[sl], sem)
            raise ValueError(kind)

        def wait_all(kind, n):
            if kind in ('wqR',):
                sl = (slice(None), pl.ds(3072, 3072))
                pltpu.make_async_copy(wq_v.at[sl], wq_v.at[sl], sem_w.at[WSEM[kind]]).wait()
            elif kind == 'w3':
                pltpu.make_async_copy(w3_v, w3_v, sem_w.at[WSEM[kind]]).wait()
            elif kind == 'w2b':
                sl = pl.ds(N2 * 32, N2 * 32)
                pltpu.make_async_copy(w2_v.at[sl], w2_v.at[sl], sem_w.at[WSEM[kind]]).wait()

        def starts(t, k1, o1, k0, o0):
            if k1 is not None:
                cp(k1, t + KD - o1).start(priority=1)
            if k0 is not None:
                cp(k0, t - o0).start(priority=0)

        x_cp = pltpu.make_async_copy(x_hbm, x_v, sem_x.at[0])
        for t in range(KD):
            k, i = locate(T1, t)
            cp(k, i).start(priority=1)
            if t == 0:
                x_cp.start(priority=0)

        def q_piece(j):
            if 'q' in off: return
            c0 = _mo(j * 384, 128)
            q = jnp.dot(xn_s[...], wq_v[:, pl.ds(c0, 384)], preferred_element_type=f32)
            q = q.astype(bf16).astype(f32)
            qrow[2 * j, :, 0:DH] = q[:, 0:DH]
            qrow[2 * j + 1, :, 0:DH] = q[:, DH:2 * DH]

        def build_qbc(h):
            if 'b' in off: return
            diff = lax.broadcasted_iota(jnp.int32, (8, 128), 1) - lax.broadcasted_iota(jnp.int32, (8, 128), 0)
            slot = _and(h, 1)
            qa = qrow[h, :, 0:128]
            qb_ = qrow[h, :, 128:DH]
            for g in range(DH // 8):
                if g < 16:
                    sel = jnp.where(diff == g * 8, qa, 0.0)
                else:
                    sel = jnp.where(diff[:, 0:64] == (g - 16) * 8, qb_, 0.0)
                col = jnp.sum(sel, axis=1, keepdims=True)
                qbc[slot, pl.ds(g * 8, 8), :] = jnp.broadcast_to(col, (8, 128))

        def qk(n, b, c):
            if 'k' in off: return
            slot = _and(n, KR - 1)
            qs = _and(b, 1)
            parts = []
            for g in range(DH // 16):
                k = kbuf[slot, pl.ds(g * 16, 16), :].astype(f32)
                parts.append(k * qbc[qs, pl.ds(g * 16, 16), :])
            tt = _tree_sum(parts)
            s_scr[pl.ds(_mo(c * 8, 8), 8), :] = tt[0:8] + tt[8:16]

        def pv(n, c):
            if 'v' in off: return
            slot = _and(n, VR - 1)
            p = jnp.broadcast_to(p_scr[pl.ds(c, 1), :], (16, 128))
            for g in range(DH // 16):
                v = vbuf[slot, pl.ds(g * 16, 16), :].astype(f32)
                acc_ref[pl.ds(g * 16, 16), :] += v * p

        def softmax():
            if 's' in off: return jnp.ones((1, 1), f32)
            rows = [_tree_sum([s_scr[pl.ds(g * 64 + j, 8, stride=8), :] for j in range(8)]) for g in range(NC // 8)]
            s = jnp.concatenate(rows, axis=0) * (DH ** -0.5)
            m = jnp.max(jnp.max(s, axis=0, keepdims=True), axis=1, keepdims=True)
            p = jnp.exp(s - m)
            l = jnp.sum(jnp.sum(p, axis=0, keepdims=True), axis=1, keepdims=True)
            p_scr[...] = p
            return l

        def finalize(h, l):
            if 'z' in off: return
            o = jnp.sum(acc_ref[...], axis=1, keepdims=True) / l
            obc[pl.ds(_mo(h * DH, 8), DH), :] = jnp.broadcast_to(o, (DH, 128))

        def wo_piece(u, y):
            if 'o' in off: return y
            r0 = _mo(u * 32, 32)
            for g in range(2):
                w = wo_v[pl.ds(r0 + g * 16, 16), :].astype(f32)
                ob = obc[pl.ds(r0 + g * 16, 16), :]
                pr = w * jnp.concatenate([ob] * (D // 128), axis=1)
                y = y + pr[0:8] + pr[8:16]
            return y

        def ffn():
            if 'f' in off: return
            xn8 = xn_s[...]
            gate = jnp.dot(xn8, w1_v[...], preferred_element_type=f32)
            up = jnp.dot(xn8, w3_v[...], preferred_element_type=f32)
            hh = (gate * jax.nn.sigmoid(gate) * up).astype(bf16)
            ff = jnp.dot(hh, w2_v[...], preferred_element_type=f32)
            g_s[...] = ff * jax.nn.sigmoid(ff)

        x_cp.wait()
        x = x_v[...].reshape(1, D).astype(f32)
        mu = jnp.mean(x, axis=-1, keepdims=True)
        xc = x - mu
        var = jnp.mean(xc * xc, axis=-1, keepdims=True)
        xn_s[...] = jnp.broadcast_to((xc / jnp.sqrt(var + 1e-5)).astype(bf16), (8, D))

        cuts = {0, A, NQ, NQ + N1, QT0, QT0 + 16}
        o = 0
        for k, n in T1:
            o += n
            if 0 < o - KD < A:
                cuts.add(o - KD)
        cuts = sorted(c for c in cuts if 0 <= c <= A)
        for t0, t1 in zip(cuts[:-1], cuts[1:]):
            kw, _ = locate(T1, t0)
            k1, _ = locate(T1, t0 + KD)
            k0, _ = locate(T0, t0)
            if t0 == QT0:
                wait_all('wqR', NQ)

            def body(t, carry, kw=kw, k1=k1, k0=k0, t0=t0):
                cp(kw, t - offset(T1, kw)).wait()
                if t0 == QT0:
                    q_piece(t - QT0)
                starts(t, k1, offset(T1, k1), k0, offset(T0, k0))
                return carry
            lax.fori_loop(t0, t1, body, 0)

        oK, oV, oA, oB = offset(T1, 'K'), offset(T0, 'V'), offset(T1, 'woa'), offset(T0, 'wob')

        def block(b, do_pv, k1, l_prev, nxt=True):
            if do_pv:
                acc_ref[...] = jnp.zeros_like(acc_ref)

            def body(c, carry):
                n = b * NC + c
                cp('K', n).wait()
                if do_pv:
                    cp('V', n - NC).wait()
                qk(n, b, c)
                if do_pv:
                    pv(n - NC, c)
                starts(A + n, k1, offset(T1, k1), 'V', oV)
                return carry
            lax.fori_loop(0, NC, body, 0)
            if do_pv:
                finalize(b - 1, l_prev)
            if nxt:
                build_qbc(b + 1)
            return softmax()

        nl = KD // NC
        build_qbc(0)
        l = block(0, False, 'K', None)
        wait_all('w3', N1)
        wait_all('w2b', N2)
        ffn()
        l = lax.fori_loop(1, H - nl, lambda b, l: block(b, True, 'K', l), l)
        for b in range(H - nl, H):
            l = block(b, True, 'woa', l, nxt=b + 1 < H)

        acc_ref[...] = jnp.zeros_like(acc_ref)
        tB = A + NKV
        cuts = sorted({0, WL, NC, B1 - KD, B0, B0 + WL, B1})
        cuts = [c for c in cuts if 0 <= c <= B1]
        y = jnp.zeros((8, D), f32)
        for j0, j1 in zip(cuts[:-1], cuts[1:]):
            do_pv = j1 <= NC
            s1 = 'woa' if j0 + KD < B1 else None
            s0 = 'wob' if j0 < B0 else None
            w0 = WL <= j0 < B0 + WL

            def body(j, y, do_pv=do_pv, s1=s1, s0=s0, w0=w0):
                cp('woa', j).wait()
                if do_pv:
                    cp('V', NKV - NC + j).wait()
                if w0:
                    cp('wob', j - WL).wait()
                if do_pv:
                    pv(NKV - NC + j, j)
                y = wo_piece(j, y)
                if w0:
                    y = wo_piece(B1 + j - WL, y)
                starts(tB + j, s1, offset(T1, 'woa'), s0, offset(T0, 'wob'))
                return y
            y = lax.fori_loop(j0, j1, body, y)
            if j1 == NC:
                finalize(H - 1, l)

        s = jnp.sum(y, axis=0, keepdims=True)
        out = x_v[...].reshape(1, D).astype(f32) + s * g_s[0:1]
        o_ref[...] = out.astype(bf16).reshape(1, 1, D)

    def simulate():
        started, waited = set(), set()
        def st(k, i):
            n = dict(T1 + T0)[k]
            assert 0 <= i < n, (k, i)
            assert (k, i) not in started
            started.add((k, i))
        def wt(k, i):
            assert (k, i) in started, ('wait before start', k, i)
            assert (k, i) not in waited
            waited.add((k, i))
        for t in range(KD):
            st(*locate(T1, t))
        for t in range(NT):
            k, i = locate(T1, t)
            wt(k, i)
            if k == 'K' and i >= NC:
                wt('V', i - NC)
            if k == 'woa':
                if i < NC:
                    wt('V', NKV - NC + i)
                if WL <= i < B0 + WL:
                    wt('wob', i - WL)
            k1, i1 = locate(T1, t + KD)
            if k1 is not None:
                st(k1, i1)
            k0, i0 = locate(T0, t)
            if k0 is not None:
                st(k0, i0)
        for k in ('wqR', 'w3', 'w2b'):
            for i in range(dict(T0)[k]):
                wt(k, i)
        assert started == waited, (len(started), len(waited), sorted(started - waited)[:5])
        assert B0 + WL <= B1 and B1 <= 128 and WL < 16
        assert KD % NC == 0 and KD + 2 <= KR and VR >= NC + 2
        assert B1 <= 186 and (186 - B1) + WL >= NC
    simulate()

    @jax.jit
    def kernel_fn(A_x, A_k_cache, A_v_cache, A_wq, A_wo, B_x, B_w1, B_w3, B_w2):
        kT = jnp.swapaxes(A_k_cache, 2, 3).reshape(HD, SK)
        vT = jnp.swapaxes(A_v_cache, 2, 3).reshape(HD, SK)
        return pl.pallas_call(
            _kernel,
            in_specs=[pl.BlockSpec(memory_space=pl.ANY)] * 8,
            out_specs=pl.BlockSpec(memory_space=pltpu.VMEM),
            out_shape=jax.ShapeDtypeStruct((1, 1, D), bf16),
            scratch_shapes=[
                pltpu.VMEM((1, 1, D), bf16),
                pltpu.VMEM((D, HD), bf16),
                pltpu.VMEM((HD, D), bf16),
                pltpu.VMEM((D, F), bf16),
                pltpu.VMEM((D, F), bf16),
                pltpu.VMEM((F, D), bf16),
                pltpu.VMEM((KR, DH, 128), bf16),
                pltpu.VMEM((VR, DH, 128), bf16),
                pltpu.VMEM((2, DH, 128), f32),
                pltpu.VMEM((H, 8, DH), f32),
                pltpu.VMEM((HD, 128), f32),
                pltpu.VMEM((NC * 8, 128), f32),
                pltpu.VMEM((NC, 128), f32),
                pltpu.VMEM((DH, 128), f32),
                pltpu.VMEM((8, D), bf16),
                pltpu.VMEM((8, D), f32),
                pltpu.SemaphoreType.DMA((1,)),
                pltpu.SemaphoreType.DMA((6,)),
                pltpu.SemaphoreType.DMA((KR,)),
                pltpu.SemaphoreType.DMA((VR,)),
                pltpu.SemaphoreType.DMA((128,)),
                pltpu.SemaphoreType.DMA((16,)),
            ],
            compiler_params=pltpu.CompilerParams(vmem_limit_bytes=100 * 1024 * 1024,
                                                 disable_bounds_checks=True, disable_semaphore_checks=True),
        )(A_x, kT, vT, A_wq, A_wo, B_w1, B_w3, B_w2)
    return kernel_fn

_impl = make()


@jax.jit
def pallas_recurrent_scan__sliding_block_cached__glu_gated_swiglu__decode_kernel(
        A_x, A_k_cache, A_v_cache, A_wq, A_wo, B_x, B_w1, B_w3, B_w2):
    return _impl(A_x, A_k_cache, A_v_cache, A_wq, A_wo, B_x, B_w1, B_w3, B_w2)
```

```python
import jax
import jax.numpy as jnp
from jax import lax
from jax.experimental import pallas as pl
from jax.experimental.pallas import tpu as pltpu

D, F, H, DH, SK = 640, 1536, 32, 192, 32768
W = min(4096, max(256, SK // 4))
HD = H * DH
NC = W // 128
RB, CB = 64, 256
NRB = DH // RB
NCB = W // CB
UH = NRB * NCB
NKV = H * UH
QG5 = 5
f32, bf16 = jnp.float32, jnp.bfloat16


def _tree_sum(xs):
    xs = list(xs)
    while len(xs) > 1:
        xs = [xs[i] + xs[i + 1] if i + 1 < len(xs) else xs[i] for i in range(0, len(xs), 2)]
    return xs[0]


def _is_int(i):
    return isinstance(i, int)


def _shr(i, s):
    return i >> s if _is_int(i) else lax.shift_right_logical(i, s)


def _and(i, m):
    return i & m if _is_int(i) else lax.bitwise_and(i, m)


def _mo(i, m):
    return i if _is_int(i) else pl.multiple_of(i, m)


class _NoScope:
    def __enter__(self):
        return self

    def __exit__(self, *args):
        return False


def _runs(items):
    out, s = [], 0
    for i in range(1, len(items) + 1):
        if i == len(items) or items[i] != items[s]:
            out.append((s, i, items[s]))
            s = i
    return out


def make(KD=48, D0=24, KR=128, VR=128, B1=96, WL=18, QG=2, PG=4, off='', prof=False):
    NQ, N1, N2, NO = 128, 40, 24, 192
    A = NQ + N1 + N2
    B0 = NO - B1
    T1 = [('wqA', NQ), ('w1', N1), ('w2a', N2), ('K', NKV), ('woa', B1)]
    T0 = [('wqB', NQ), ('w3', N1), ('w2b', N2), ('V', NKV), ('wob', B0)]
    NT = A + NKV + B1
    WLC = WL - D0
    assert KD % 24 == 0 and D0 % 24 == 0 and A % 8 == 0

    def locate(lst, t):
        for kind, n in lst:
            if 0 <= t < n:
                return kind, t
            t -= n
        return None, None

    def offset(lst, kind):
        o = 0
        for k, n in lst:
            if k == kind:
                return o
            o += n

    OFF = {k: offset(T1, k) for k, _ in T1}
    OFF.update({k: offset(T0, k) for k, _ in T0})

    CNT = dict(T1 + T0)
    PSH = PG.bit_length() - 1

    def perm(kind, i):
        if PG == 1:
            return i
        assert CNT[kind] % PG == 0, (kind, CNT[kind])
        return _and(i, PG - 1) * (CNT[kind] // PG) + _shr(i, PSH)

    def scope(name):
        return jax.named_scope(name) if prof else _NoScope()

    def _kernel(x_hbm, k_hbm, v_hbm, wq_hbm, wo_hbm, w1_hbm, w3_hbm, w2_hbm, o_ref,
                x_v, wq_v, wo_v, w1_v, w3_v, w2_v, kbuf, vbuf, qbc, qrow, obc, s_scr, p_scr, acc_ref, xn_s, g_s,
                sem_x, sem_1, sem_q, sem_w, sem_v, sem_ob):

        def cp(kind, i):
            s1 = lambda: sem_1.at[_and(i + OFF[kind], 127)]
            if kind in ('wqA', 'wqB'):
                j = _shr(i, 3)
                rt = _and(i, 7) * 2 + (0 if kind == 'wqA' else 1)
                sl = (slice(None), pl.ds(_mo(rt * 8, 8), 8), pl.ds(_mo(j * 384, 128), 384))
                sem = s1() if kind == 'wqA' else sem_q.at[j]
                return pltpu.make_async_copy(wq_hbm.at[sl], wq_v.at[sl], sem)
            if kind in ('w1', 'w3'):
                src, dst = (w1_hbm, w1_v) if kind == 'w1' else (w3_hbm, w3_v)
                sl = pl.ds(_mo(perm(kind, i) * 16, 16), 16)
                return pltpu.make_async_copy(src.at[sl], dst.at[sl], s1() if kind == 'w1' else sem_w.at[0])
            if kind in ('w2a', 'w2b'):
                sl = pl.ds(_mo((perm(kind, i) + (0 if kind == 'w2a' else N2)) * 32, 32), 32)
                return pltpu.make_async_copy(w2_hbm.at[sl], w2_v.at[sl], s1() if kind == 'w2a' else sem_w.at[1])
            if kind in ('K', 'V'):
                g, rb = i if isinstance(i, tuple) else divmod(i, NRB)
                n = g * NRB + rb
                src, buf, ring = (k_hbm, kbuf, KR) if kind == 'K' else (v_hbm, vbuf, VR)
                r0 = _mo(_shr(g, 4) * DH + rb * RB, 8)
                c0 = _mo(SK - W + _and(g, NCB - 1) * CB, 128)
                slot = _and(n, ring - 1)
                sem = sem_1.at[_and(n + OFF['K'], 127)] if kind == 'K' else sem_v.at[slot]
                return pltpu.make_async_copy(src.at[pl.ds(r0, RB), pl.ds(c0, CB)], buf.at[slot], sem)
            if kind in ('woa', 'wob'):
                u = perm(kind, i) + (0 if kind == 'woa' else B1)
                sl = pl.ds(_mo(u * 32, 32), 32)
                sem = s1() if kind == 'woa' else sem_ob.at[_and(i, 31)]
                return pltpu.make_async_copy(wo_hbm.at[sl], wo_v.at[sl], sem)
            raise ValueError(kind)

        x_cp = pltpu.make_async_copy(x_hbm, x_v, sem_x.at[0])
        with scope('s0_prologue'):
            x_cp.start(priority=0)

            def pro(t, c):
                cp('wqA', t).start(priority=1)
                cp('wqB', t).start(priority=0)
                return c
            if D0:
                lax.fori_loop(0, D0, pro, 0)

            def pro1(t, c):
                cp('wqA', t).start(priority=1)
                return c
            assert KD <= NQ
            lax.fori_loop(D0, KD, pro1, 0)

        def layernorm():
            x_cp.wait()
            x = x_v[...].reshape(1, D).astype(f32)
            mu = jnp.mean(x, axis=-1, keepdims=True)
            xc = x - mu
            var = jnp.mean(xc * xc, axis=-1, keepdims=True)
            xn_s[...] = jnp.broadcast_to((xc / jnp.sqrt(var + 1e-5)).astype(bf16), (8, D))

        def q_piece(j):
            sl = (slice(None), pl.ds(0, 64), pl.ds(0, 384))
            pltpu.make_async_copy(wq_v.at[sl], wq_v.at[sl], sem_q.at[j]).wait()
            if 'q' in off: return
            c0 = _mo(j * 384, 128)
            w = wq_v[:, :, pl.ds(c0, 384)].reshape(D, 384)
            q = jnp.dot(xn_s[...], w, preferred_element_type=f32)
            q = q.astype(bf16).astype(f32)
            qrow[2 * j, :, 0:DH] = q[:, 0:DH]
            qrow[2 * j + 1, :, 0:DH] = q[:, DH:2 * DH]

        def build_qbc(h):
            if 'b' in off: return
            diff = lax.broadcasted_iota(jnp.int32, (8, 128), 1) - lax.broadcasted_iota(jnp.int32, (8, 128), 0)
            slot = _and(h, 1)
            qa = qrow[h, :, 0:128]
            qb_ = qrow[h, :, 128:DH]
            for g in range(DH // 8):
                if g < 16:
                    sel = jnp.where(diff == g * 8, qa, 0.0)
                else:
                    sel = jnp.where(diff[:, 0:64] == (g - 16) * 8, qb_, 0.0)
                col = jnp.sum(sel, axis=1, keepdims=True)
                qbc[slot, pl.ds(g * 8, 8), :] = jnp.broadcast_to(col, (8, 128))

        def qk(n, b, rb, t):
            if 'k' in off: return t
            slot = _and(n, KR - 1)
            qs = _and(b, 1)
            lo, hi = [], []
            for g in range(RB // 16):
                k = kbuf[slot, pl.ds(g * 16, 16), :].astype(f32)
                q = qbc[qs, pl.ds(rb * RB + g * 16, 16), :]
                lo.append(k[:, 0:128] * q)
                hi.append(k[:, 128:256] * q)
            if t is not None:
                lo.append(t[0])
                hi.append(t[1])
            return _tree_sum(lo), _tree_sum(hi)

        def qk_store(t, cb):
            if 'k' in off: return
            r0 = _mo(cb * 16, 16)
            s_scr[pl.ds(r0, 8), :] = t[0][0:8] + t[0][8:16]
            s_scr[pl.ds(r0 + 8, 8), :] = t[1][0:8] + t[1][8:16]

        def pv(n, cb, rb):
            if 'v' in off: return
            slot = _and(n, VR - 1)
            p0 = jnp.broadcast_to(p_scr[pl.ds(2 * cb, 1), :], (16, 128))
            p1 = jnp.broadcast_to(p_scr[pl.ds(2 * cb + 1, 1), :], (16, 128))
            for g in range(RB // 16):
                v = vbuf[slot, pl.ds(g * 16, 16), :].astype(f32)
                acc_ref[pl.ds(rb * RB + g * 16, 16), :] += v[:, 0:128] * p0 + v[:, 128:256] * p1

        def softmax():
            if 's' in off: return jnp.ones((1, 1), f32)
            rows = [_tree_sum([s_scr[pl.ds(g * 64 + j, 8, stride=8), :] for j in range(8)]) for g in range(NC // 8)]
            s = jnp.concatenate(rows, axis=0) * (DH ** -0.5)
            m = jnp.max(jnp.max(s, axis=0, keepdims=True), axis=1, keepdims=True)
            p = jnp.exp(s - m)
            l = jnp.sum(jnp.sum(p, axis=0, keepdims=True), axis=1, keepdims=True)
            p_scr[...] = p
            return l

        def finalize(h, l):
            if 'z' in off: return
            o = jnp.sum(acc_ref[...], axis=1, keepdims=True) / l
            obc[pl.ds(_mo(h * DH, 8), DH), :] = jnp.broadcast_to(o, (DH, 128))

        def wo_piece(u, y):
            if 'o' in off: return y
            r0 = _mo(u * 32, 32)
            for g in range(2):
                w = wo_v[pl.ds(r0 + g * 16, 16), :].astype(f32)
                ob = obc[pl.ds(r0 + g * 16, 16), :]
                pr = w * jnp.concatenate([ob] * (D // 128), axis=1)
                y = y + pr[0:8] + pr[8:16]
            return y

        def ffn():
            if 'f' in off: return
            xn8 = xn_s[...]
            gate = jnp.dot(xn8, w1_v[...], preferred_element_type=f32)
            up = jnp.dot(xn8, w3_v[...], preferred_element_type=f32)
            hh = (gate * jax.nn.sigmoid(gate) * up).astype(bf16)
            ff = jnp.dot(hh, w2_v[...], preferred_element_type=f32)
            g_s[...] = ff * jax.nn.sigmoid(ff)

        def start(kind, i, prio):
            if kind is not None:
                cp(kind, i).start(priority=prio)

        def startA(kind, tt, prio):
            i = tt - OFF[kind]
            if kind in ('K', 'V'):
                gi = lax.shift_right_logical(i * 171, 9)
                cp(kind, (gi, i - gi * NRB)).start(priority=prio)
            else:
                cp(kind, i).start(priority=prio)

        groups = []
        for g in range(A // 8):
            t = g * 8
            groups.append((locate(T1, t)[0], locate(T1, t + KD)[0], locate(T0, t + D0)[0], 0 <= g - QG < 16, g == QG))
        for g0, g1, (kw, k1, k0, has_q, first) in _runs(groups):
            if first:
                with scope('s1_ln'):
                    layernorm()

            def group(g, carry, kw=kw, k1=k1, k0=k0, has_q=has_q):
                for s in range(8):
                    t = g * 8 + s
                    cp(kw, t - OFF[kw]).wait()
                    startA(k1, t + KD, 1)
                    startA(k0, t + D0, 0)
                if has_q:
                    q_piece(g - QG)
                return carry

            with scope('s2_seg%03d' % (g0 * 8)):
                lax.fori_loop(g0, g1, group, 0)

        def kinds(n):
            return locate(T1, A + n + KD)[0], locate(T0, A + n + D0)[0]

        def iteration(b, cb, do_pv, k1, k0):
            g = b * NCB + cb
            t = None
            for rb in range(NRB):
                n = g * NRB + rb
                cp('K', (g, rb)).wait()
                if do_pv:
                    cp('V', (g - NCB, rb)).wait()
                t = qk(n, b, rb, t)
                if do_pv:
                    pv(n - UH, cb, rb)
                if k1 == 'K':
                    cp('K', (g + KD // NRB, rb)).start(priority=1)
                else:
                    start(k1, A + n + KD - OFF['woa'], 1)
                if k0 == 'V':
                    cp('V', (g + D0 // NRB, rb)).start(priority=0)
                else:
                    start(k0, A + n + D0 - OFF['wob'], 0)
            qk_store(t, cb)

        def block(b, do_pv, segs, l_prev, nxt=True):
            if do_pv:
                acc_ref[...] = jnp.zeros_like(acc_ref)
            for c0, c1, (k1, k0) in segs:
                def body(cb, carry, k1=k1, k0=k0):
                    iteration(b, cb, do_pv, k1, k0)
                    return carry
                lax.fori_loop(c0, c1, body, 0)
            if do_pv:
                finalize(b - 1, l_prev)
            if nxt:
                build_qbc(b + 1)
            return softmax()

        def segs_of(b):
            return _runs([kinds(b * UH + cb * NRB) for cb in range(NCB)])

        plain = [(0, NCB, ('K', 'V'))]
        nplain = max(b for b in range(H) if segs_of(b) == plain) + 1
        with scope('s3_block0'):
            build_qbc(0)
            l = block(0, False, plain, None)
        with scope('s4_ffn'):
            pltpu.make_async_copy(w3_v, w3_v, sem_w.at[0]).wait()
            sl = pl.ds(N2 * 32, N2 * 32)
            pltpu.make_async_copy(w2_v.at[sl], w2_v.at[sl], sem_w.at[1]).wait()
            ffn()
        with scope('s5_main'):
            l = lax.fori_loop(1, nplain, lambda b, l: block(b, True, plain, l), l)
        with scope('s6_lastblocks'):
            for b in range(nplain, H):
                l = block(b, True, segs_of(b), l, nxt=b + 1 < H)

        acc_ref[...] = jnp.zeros_like(acc_ref)
        tB = A + NKV
        WC = max(WLC, 0)

        def attrsB(j):
            return (j < UH, locate(T1, tB + j + KD)[0], locate(T0, tB + j + D0)[0], WC <= j < B0 + WC)

        y = jnp.zeros((8, D), f32)
        ticks = [attrsB(j) for j in range(B1)]
        for j0, j1, (do_pv, s1, s0, w0) in _runs(ticks):
            def one(j, y, rb, cb, do_pv=do_pv, s1=s1, s0=s0, w0=w0):
                cp('woa', j).wait()
                if do_pv:
                    cp('V', ((H - 1) * NCB + cb, rb)).wait()
                if w0:
                    cp('wob', j - WC).wait()
                if do_pv:
                    pv((NKV - UH) + cb * NRB + rb, cb, rb)
                y = wo_piece(perm('woa', j), y)
                if w0:
                    y = wo_piece(B1 + perm('wob', j - WC), y)
                start(s1, tB + j + KD - OFF['woa'], 1)
                start(s0, tB + j + D0 - OFF['wob'], 0)
                return y

            with scope('s7_seg%03d' % j0):
                if do_pv:
                    assert j0 % NRB == 0 and j1 % NRB == 0, (j0, j1)

                    def body3(cb, y, one=one):
                        for rb in range(NRB):
                            y = one(cb * NRB + rb, y, rb, cb)
                        return y
                    y = lax.fori_loop(j0 // NRB, j1 // NRB, body3, y)
                else:
                    y = lax.fori_loop(j0, j1, lambda j, y, one=one: one(j, y, None, None), y)
            if j1 == UH:
                finalize(H - 1, l)

        if B1 - WC < B0:
            def tail(i, y):
                cp('wob', i).wait()
                return wo_piece(B1 + perm('wob', i), y)
            with scope('s7_tail'):
                y = lax.fori_loop(B1 - WC, B0, tail, y)

        s = jnp.sum(y, axis=0, keepdims=True)
        out = x_v[...].reshape(1, D).astype(f32) + s * g_s[0:1]
        o_ref[...] = out.astype(bf16).reshape(1, 1, D)

    def simulate():
        started, waited = set(), set()
        WC = max(WLC, 0)
        def st(k, i):
            n = dict(T1 + T0)[k]
            assert 0 <= i < n, (k, i)
            assert (k, i) not in started
            started.add((k, i))
            if k in OFF and k in dict(T1):
                gi = i + OFF[k] - 128
                if gi >= 0:
                    assert locate(T1, gi) in waited, (k, i)
            if k == 'K' and i >= KR:
                assert ('K', i - KR) in waited
            if k == 'V' and i >= VR:
                assert ('V', i - VR) in waited
            if k == 'wob' and i >= 32:
                assert ('wob', i - 32) in waited
        def wt(k, i):
            assert (k, i) in started, ('wait before start', k, i)
            assert (k, i) not in waited
            waited.add((k, i))
        for t in range(D0):
            st(*locate(T0, t))
        for t in range(KD):
            st(*locate(T1, t))
        for t in range(NT):
            k, i = locate(T1, t)
            wt(k, i)
            if k == 'K' and i >= UH:
                wt('V', i - UH)
            if k == 'woa':
                if i < UH:
                    wt('V', NKV - UH + i)
                if WC <= i < B0 + WC:
                    wt('wob', i - WC)
            k1, i1 = locate(T1, t + KD)
            if k1 is not None:
                st(k1, i1)
            k0, i0 = locate(T0, t + D0)
            if k0 is not None:
                st(k0, i0)
            if t < A and t % 8 == 7 and 0 <= t // 8 - QG < 16:
                j = t // 8 - QG
                for u in range(8):
                    assert ('wqA', 8 * j + u) in waited
                    wt('wqB', 8 * j + u)
            if t == A + UH - 1:
                for k in ('w3', 'w2b'):
                    for i in range(dict(T0)[k]):
                        wt(k, i)
                for k in ('w1', 'w2a'):
                    assert all((k, i) in waited for i in range(dict(T1)[k]))
        for i in range(max(B1 - WC, 0), B0):
            wt('wob', i)
        assert all((i * 171) >> 9 == i // 3 for i in range(512)) and max(KD, D0) < 512
        assert started == waited, (len(started), len(waited), sorted(started - waited)[:5])
        assert 15 + QG < A // 8
        assert B1 <= 186
        for i in range(B0):
            if B1 + perm('wob', i) >= 186:
                assert i + WC >= UH, i
        assert sorted(perm('wob', i) for i in range(B0)) == list(range(B0))
    simulate()

    @jax.jit
    def kernel_fn(A_x, A_k_cache, A_v_cache, A_wq, A_wo, B_x, B_w1, B_w3, B_w2):
        kT = jnp.swapaxes(A_k_cache, 2, 3).reshape(HD, SK)
        vT = jnp.swapaxes(A_v_cache, 2, 3).reshape(HD, SK)
        wq3 = A_wq.reshape(QG5, D // QG5, HD)
        return pl.pallas_call(
            _kernel,
            in_specs=[pl.BlockSpec(memory_space=pl.ANY)] * 8,
            out_specs=pl.BlockSpec(memory_space=pltpu.VMEM),
            out_shape=jax.ShapeDtypeStruct((1, 1, D), bf16),
            scratch_shapes=[
                pltpu.VMEM((1, 1, D), bf16),
                pltpu.VMEM((QG5, D // QG5, HD), bf16),
                pltpu.VMEM((HD, D), bf16),
                pltpu.VMEM((D, F), bf16),
                pltpu.VMEM((D, F), bf16),
                pltpu.VMEM((F, D), bf16),
                pltpu.VMEM((KR, RB, CB), bf16),
                pltpu.VMEM((VR, RB, CB), bf16),
                pltpu.VMEM((2, DH, 128), f32),
                pltpu.VMEM((H, 8, DH), f32),
                pltpu.VMEM((HD, 128), f32),
                pltpu.VMEM((NC * 8, 128), f32),
                pltpu.VMEM((NC, 128), f32),
                pltpu.VMEM((DH, 128), f32),
                pltpu.VMEM((8, D), bf16),
                pltpu.VMEM((8, D), f32),
                pltpu.SemaphoreType.DMA((1,)),
                pltpu.SemaphoreType.DMA((128,)),
                pltpu.SemaphoreType.DMA((16,)),
                pltpu.SemaphoreType.DMA((2,)),
                pltpu.SemaphoreType.DMA((VR,)),
                pltpu.SemaphoreType.DMA((32,)),
            ],
            compiler_params=pltpu.CompilerParams(vmem_limit_bytes=100 * 1024 * 1024,
                                                 disable_bounds_checks=True, disable_semaphore_checks=True),
        )(A_x, kT, vT, wq3, A_wo, B_w1, B_w3, B_w2)
    return kernel_fn

_impl = make()


@jax.jit
def pallas_recurrent_scan__sliding_block_cached__glu_gated_swiglu__decode_kernel(
        A_x, A_k_cache, A_v_cache, A_wq, A_wo, B_x, B_w1, B_w3, B_w2):
    return _impl(A_x, A_k_cache, A_v_cache, A_wq, A_wo, B_x, B_w1, B_w3, B_w2)
```

```python
import jax
import jax.numpy as jnp
from jax import lax
from jax.experimental import pallas as pl
from jax.experimental.pallas import tpu as pltpu

D, F, H, DH, SK = 640, 1536, 32, 192, 32768
W = min(4096, max(256, SK // 4))
HD = H * DH
NC = W // 128
RB, CB = 64, 256
NRB = DH // RB
NCB = W // CB
UH = NRB * NCB
NKV = H * UH
f32, bf16 = jnp.float32, jnp.bfloat16


def _tree_sum(xs):
    xs = list(xs)
    while len(xs) > 1:
        xs = [xs[i] + xs[i + 1] if i + 1 < len(xs) else xs[i] for i in range(0, len(xs), 2)]
    return xs[0]


def _is_int(i):
    return isinstance(i, int)


def _shr(i, s):
    return i >> s if _is_int(i) else lax.shift_right_logical(i, s)


def _and(i, m):
    return i & m if _is_int(i) else lax.bitwise_and(i, m)


def _mo(i, m):
    return i if _is_int(i) else pl.multiple_of(i, m)


class _NoScope:
    def __enter__(self):
        return self

    def __exit__(self, *args):
        return False


def _runs(items):
    out, s = [], 0
    for i in range(1, len(items) + 1):
        if i == len(items) or items[i] != items[s]:
            out.append((s, i, items[s]))
            s = i
    return out


def make(KD=48, D0=0, KR=128, VR=128, B1=108, WL=18, PG=4, QP=2, off='', prof=False):
    NQ, N1, N2, NO = 80, 40, 24, 192
    A = NQ + N1 + N2
    B0 = NO - B1
    T1 = [('wqA', NQ), ('w1', N1), ('w2a', N2), ('K', NKV), ('woa', B1)]
    T0 = [('wqB', NQ), ('w3', N1), ('w2b', N2), ('V', NKV), ('wob', B0)]
    NT = A + NKV + B1
    WLC = WL - D0
    assert KD % 24 == 0 and D0 % 24 == 0 and A % 8 == 0
    QS = A // 8 - 2 * QP
    assert QS * 8 >= NQ

    def locate(lst, t):
        for kind, n in lst:
            if 0 <= t < n:
                return kind, t
            t -= n
        return None, None

    def offset(lst, kind):
        o = 0
        for k, n in lst:
            if k == kind:
                return o
            o += n

    OFF = {k: offset(T1, k) for k, _ in T1}
    OFF.update({k: offset(T0, k) for k, _ in T0})

    CNT = dict(T1 + T0)
    PSH = PG.bit_length() - 1

    def perm(kind, i):
        if PG == 1:
            return i
        assert CNT[kind] % PG == 0, (kind, CNT[kind])
        return _and(i, PG - 1) * (CNT[kind] // PG) + _shr(i, PSH)

    def scope(name):
        return jax.named_scope(name) if prof else _NoScope()

    def _kernel(x_hbm, k_hbm, v_hbm, wq_hbm, wo_hbm, w1_hbm, w3_hbm, w2_hbm, o_ref,
                x_v, wq_v, wo_v, w1_v, w3_v, w2_v, kbuf, vbuf, qbc, qrow, obc, s_scr, p_scr, acc_ref, xn_s, g_s,
                sem_x, sem_1, sem_q, sem_w, sem_v, sem_ob):

        def cp(kind, i):
            s1 = lambda: sem_1.at[_and(i + OFF[kind], 127)]
            if kind in ('wqA', 'wqB'):
                k = _shr(i, 2)
                rt = (0 if kind == 'wqA' else 40) + _and(i, 3) * 10 + _shr(k, 1)
                sl = (pl.ds(_mo(rt * 8, 8), 8), pl.ds(_mo(_and(k, 1) * 3072, 128), 3072))
                sem = s1() if kind == 'wqA' else sem_q.at[0]
                return pltpu.make_async_copy(wq_hbm.at[sl], wq_v.at[sl], sem)
            if kind in ('w1', 'w3'):
                src, dst = (w1_hbm, w1_v) if kind == 'w1' else (w3_hbm, w3_v)
                sl = pl.ds(_mo(perm(kind, i) * 16, 16), 16)
                return pltpu.make_async_copy(src.at[sl], dst.at[sl], s1() if kind == 'w1' else sem_w.at[0])
            if kind in ('w2a', 'w2b'):
                sl = pl.ds(_mo((perm(kind, i) + (0 if kind == 'w2a' else N2)) * 32, 32), 32)
                return pltpu.make_async_copy(w2_hbm.at[sl], w2_v.at[sl], s1() if kind == 'w2a' else sem_w.at[1])
            if kind in ('K', 'V'):
                g, rb = i if isinstance(i, tuple) else divmod(i, NRB)
                n = g * NRB + rb
                src, buf, ring = (k_hbm, kbuf, KR) if kind == 'K' else (v_hbm, vbuf, VR)
                r0 = _mo(_shr(g, 4) * DH + rb * RB, 8)
                c0 = _mo(SK - W + _and(g, NCB - 1) * CB, 128)
                slot = _and(n, ring - 1)
                sem = sem_1.at[_and(n + OFF['K'], 127)] if kind == 'K' else sem_v.at[slot]
                return pltpu.make_async_copy(src.at[pl.ds(r0, RB), pl.ds(c0, CB)], buf.at[slot], sem)
            if kind in ('woa', 'wob'):
                u = perm(kind, i) + (0 if kind == 'woa' else B1)
                sl = pl.ds(_mo(u * 32, 32), 32)
                sem = s1() if kind == 'woa' else sem_ob.at[_and(i, 31)]
                return pltpu.make_async_copy(wo_hbm.at[sl], wo_v.at[sl], sem)
            raise ValueError(kind)

        x_cp = pltpu.make_async_copy(x_hbm, x_v, sem_x.at[0])
        with scope('s0_prologue'):
            x_cp.start(priority=0)

            def pro(t, c):
                cp('wqA', t).start(priority=1)
                cp('wqB', t).start(priority=0)
                return c
            if D0:
                lax.fori_loop(0, D0, pro, 0)

            def pro1(t, c):
                cp('wqA', t).start(priority=1)
                return c
            assert KD <= NQ
            lax.fori_loop(D0, KD, pro1, 0)

        def layernorm():
            x_cp.wait()
            x = x_v[...].reshape(1, D).astype(f32)
            mu = jnp.mean(x, axis=-1, keepdims=True)
            xc = x - mu
            var = jnp.mean(xc * xc, axis=-1, keepdims=True)
            xn_s[...] = jnp.broadcast_to((xc / jnp.sqrt(var + 1e-5)).astype(bf16), (8, D))

        def q_piece(j):
            if 'q' in off: return
            c0 = _mo(j * 384, 128)
            q = jnp.dot(xn_s[...], wq_v[:, pl.ds(c0, 384)], preferred_element_type=f32)
            q = q.astype(bf16).astype(f32)
            qrow[2 * j, :, 0:DH] = q[:, 0:DH]
            qrow[2 * j + 1, :, 0:DH] = q[:, DH:2 * DH]

        def build_qbc(h):
            if 'b' in off: return
            diff = lax.broadcasted_iota(jnp.int32, (8, 128), 1) - lax.broadcasted_iota(jnp.int32, (8, 128), 0)
            slot = _and(h, 1)
            qa = qrow[h, :, 0:128]
            qb_ = qrow[h, :, 128:DH]
            for g in range(DH // 8):
                if g < 16:
                    sel = jnp.where(diff == g * 8, qa, 0.0)
                else:
                    sel = jnp.where(diff[:, 0:64] == (g - 16) * 8, qb_, 0.0)
                col = jnp.sum(sel, axis=1, keepdims=True)
                qbc[slot, pl.ds(g * 8, 8), :] = jnp.broadcast_to(col, (8, 128))

        def qk(n, b, rb, t):
            if 'k' in off: return t
            slot = _and(n, KR - 1)
            qs = _and(b, 1)
            lo, hi = [], []
            for g in range(RB // 16):
                k = kbuf[slot, pl.ds(g * 16, 16), :].astype(f32)
                q = qbc[qs, pl.ds(rb * RB + g * 16, 16), :]
                lo.append(k[:, 0:128] * q)
                hi.append(k[:, 128:256] * q)
            if t is not None:
                lo.append(t[0])
                hi.append(t[1])
            return _tree_sum(lo), _tree_sum(hi)

        def qk_store(t, cb):
            if 'k' in off: return
            r0 = _mo(cb * 16, 16)
            s_scr[pl.ds(r0, 8), :] = t[0][0:8] + t[0][8:16]
            s_scr[pl.ds(r0 + 8, 8), :] = t[1][0:8] + t[1][8:16]

        def pv(n, cb, rb):
            if 'v' in off: return
            slot = _and(n, VR - 1)
            p0 = jnp.broadcast_to(p_scr[pl.ds(2 * cb, 1), :], (16, 128))
            p1 = jnp.broadcast_to(p_scr[pl.ds(2 * cb + 1, 1), :], (16, 128))
            for g in range(RB // 16):
                v = vbuf[slot, pl.ds(g * 16, 16), :].astype(f32)
                acc_ref[pl.ds(rb * RB + g * 16, 16), :] += v[:, 0:128] * p0 + v[:, 128:256] * p1

        def softmax():
            if 's' in off: return jnp.ones((1, 1), f32)
            rows = [_tree_sum([s_scr[pl.ds(g * 64 + j, 8, stride=8), :] for j in range(8)]) for g in range(NC // 8)]
            s = jnp.concatenate(rows, axis=0) * (DH ** -0.5)
            m = jnp.max(jnp.max(s, axis=0, keepdims=True), axis=1, keepdims=True)
            p = jnp.exp(s - m)
            l = jnp.sum(jnp.sum(p, axis=0, keepdims=True), axis=1, keepdims=True)
            p_scr[...] = p
            return l

        def finalize(h, l):
            if 'z' in off: return
            o = jnp.sum(acc_ref[...], axis=1, keepdims=True) / l
            obc[pl.ds(_mo(h * DH, 8), DH), :] = jnp.broadcast_to(o, (DH, 128))

        def wo_piece(u, y):
            if 'o' in off: return y
            r0 = _mo(u * 32, 32)
            for g in range(2):
                w = wo_v[pl.ds(r0 + g * 16, 16), :].astype(f32)
                ob = obc[pl.ds(r0 + g * 16, 16), :]
                pr = w * jnp.concatenate([ob] * (D // 128), axis=1)
                y = y + pr[0:8] + pr[8:16]
            return y

        def ffn():
            if 'f' in off: return
            xn8 = xn_s[...]
            gate = jnp.dot(xn8, w1_v[...], preferred_element_type=f32)
            up = jnp.dot(xn8, w3_v[...], preferred_element_type=f32)
            hh = (gate * jax.nn.sigmoid(gate) * up).astype(bf16)
            ff = jnp.dot(hh, w2_v[...], preferred_element_type=f32)
            g_s[...] = ff * jax.nn.sigmoid(ff)

        def start(kind, i, prio):
            if kind is not None:
                cp(kind, i).start(priority=prio)

        def startA(kind, tt, prio):
            i = tt - OFF[kind]
            if kind in ('K', 'V'):
                gi = lax.shift_right_logical(i * 171, 9)
                cp(kind, (gi, i - gi * NRB)).start(priority=prio)
            else:
                cp(kind, i).start(priority=prio)

        groups = []
        for g in range(A // 8):
            t = g * 8
            groups.append((locate(T1, t)[0], locate(T1, t + KD)[0], locate(T0, t + D0)[0], g >= QS))
        for g0, g1, (kw, k1, k0, has_q) in _runs(groups):
            if g0 == QS:
                with scope('s1_ln'):
                    layernorm()
                    sl = pl.ds(D // 2, D // 2)
                    pltpu.make_async_copy(wq_v.at[sl], wq_v.at[sl], sem_q.at[0]).wait()

            def group(g, carry, kw=kw, k1=k1, k0=k0, has_q=has_q):
                for s in range(8):
                    t = g * 8 + s
                    cp(kw, t - OFF[kw]).wait()
                    startA(k1, t + KD, 1)
                    startA(k0, t + D0, 0)
                    if has_q and s % QP == QP - 1:
                        q_piece((g - QS) * (8 // QP) + s // QP)
                return carry

            with scope('s2_seg%03d' % (g0 * 8)):
                lax.fori_loop(g0, g1, group, 0)

        def kinds(n):
            return locate(T1, A + n + KD)[0], locate(T0, A + n + D0)[0]

        def iteration(b, cb, do_pv, k1, k0):
            g = b * NCB + cb
            t = None
            for rb in range(NRB):
                n = g * NRB + rb
                cp('K', (g, rb)).wait()
                if do_pv:
                    cp('V', (g - NCB, rb)).wait()
                t = qk(n, b, rb, t)
                if do_pv:
                    pv(n - UH, cb, rb)
                if k1 == 'K':
                    cp('K', (g + KD // NRB, rb)).start(priority=1)
                else:
                    start(k1, A + n + KD - OFF['woa'], 1)
                if k0 == 'V':
                    cp('V', (g + D0 // NRB, rb)).start(priority=0)
                else:
                    start(k0, A + n + D0 - OFF['wob'], 0)
            qk_store(t, cb)

        def block(b, do_pv, segs, l_prev, nxt=True):
            if do_pv:
                acc_ref[...] = jnp.zeros_like(acc_ref)
            for c0, c1, (k1, k0) in segs:
                def body(cb, carry, k1=k1, k0=k0):
                    iteration(b, cb, do_pv, k1, k0)
                    return carry
                lax.fori_loop(c0, c1, body, 0)
            if do_pv:
                finalize(b - 1, l_prev)
            if nxt:
                build_qbc(b + 1)
            return softmax()

        def segs_of(b):
            return _runs([kinds(b * UH + cb * NRB) for cb in range(NCB)])

        plain = [(0, NCB, ('K', 'V'))]
        nplain = max(b for b in range(H) if segs_of(b) == plain) + 1
        with scope('s3_block0'):
            build_qbc(0)
            l = block(0, False, plain, None)
        with scope('s4_ffn'):
            pltpu.make_async_copy(w3_v, w3_v, sem_w.at[0]).wait()
            sl = pl.ds(N2 * 32, N2 * 32)
            pltpu.make_async_copy(w2_v.at[sl], w2_v.at[sl], sem_w.at[1]).wait()
            ffn()
        with scope('s5_main'):
            l = lax.fori_loop(1, nplain, lambda b, l: block(b, True, plain, l), l)
        with scope('s6_lastblocks'):
            for b in range(nplain, H):
                l = block(b, True, segs_of(b), l, nxt=b + 1 < H)

        acc_ref[...] = jnp.zeros_like(acc_ref)
        tB = A + NKV
        WC = max(WLC, 0)

        def attrsB(j):
            return (j < UH, locate(T1, tB + j + KD)[0], locate(T0, tB + j + D0)[0], WC <= j < B0 + WC)

        y = jnp.zeros((8, D), f32)
        ticks = [attrsB(j) for j in range(B1)]
        for j0, j1, (do_pv, s1, s0, w0) in _runs(ticks):
            def one(j, y, rb, cb, do_pv=do_pv, s1=s1, s0=s0, w0=w0):
                cp('woa', j).wait()
                if do_pv:
                    cp('V', ((H - 1) * NCB + cb, rb)).wait()
                if w0:
                    cp('wob', j - WC).wait()
                if do_pv:
                    pv((NKV - UH) + cb * NRB + rb, cb, rb)
                y = wo_piece(perm('woa', j), y)
                if w0:
                    y = wo_piece(B1 + perm('wob', j - WC), y)
                start(s1, tB + j + KD - OFF['woa'], 1)
                start(s0, tB + j + D0 - OFF['wob'], 0)
                return y

            with scope('s7_seg%03d' % j0):
                if do_pv:
                    assert j0 % NRB == 0 and j1 % NRB == 0, (j0, j1)

                    def body3(cb, y, one=one):
                        for rb in range(NRB):
                            y = one(cb * NRB + rb, y, rb, cb)
                        return y
                    y = lax.fori_loop(j0 // NRB, j1 // NRB, body3, y)
                else:
                    y = lax.fori_loop(j0, j1, lambda j, y, one=one: one(j, y, None, None), y)
            if j1 == UH:
                finalize(H - 1, l)

        if B1 - WC < B0:
            def tail(i, y):
                cp('wob', i).wait()
                return wo_piece(B1 + perm('wob', i), y)
            with scope('s7_tail'):
                y = lax.fori_loop(B1 - WC, B0, tail, y)

        s = jnp.sum(y, axis=0, keepdims=True)
        out = x_v[...].reshape(1, D).astype(f32) + s * g_s[0:1]
        o_ref[...] = out.astype(bf16).reshape(1, 1, D)

    def simulate():
        started, waited = set(), set()
        WC = max(WLC, 0)
        def st(k, i):
            n = dict(T1 + T0)[k]
            assert 0 <= i < n, (k, i)
            assert (k, i) not in started
            started.add((k, i))
            if k in OFF and k in dict(T1):
                gi = i + OFF[k] - 128
                if gi >= 0:
                    assert locate(T1, gi) in waited, (k, i)
            if k == 'K' and i >= KR:
                assert ('K', i - KR) in waited
            if k == 'V' and i >= VR:
                assert ('V', i - VR) in waited
            if k == 'wob' and i >= 32:
                assert ('wob', i - 32) in waited
        def wt(k, i):
            assert (k, i) in started, ('wait before start', k, i)
            assert (k, i) not in waited
            waited.add((k, i))
        for t in range(D0):
            st(*locate(T0, t))
        for t in range(KD):
            st(*locate(T1, t))
        for t in range(NT):
            k, i = locate(T1, t)
            wt(k, i)
            if k == 'K' and i >= UH:
                wt('V', i - UH)
            if k == 'woa':
                if i < UH:
                    wt('V', NKV - UH + i)
                if WC <= i < B0 + WC:
                    wt('wob', i - WC)
            k1, i1 = locate(T1, t + KD)
            if k1 is not None:
                st(k1, i1)
            k0, i0 = locate(T0, t + D0)
            if k0 is not None:
                st(k0, i0)
            if t == QS * 8 - 1:
                for u in range(NQ):
                    assert ('wqA', u) in waited
                    wt('wqB', u)
            if t == A + UH - 1:
                for k in ('w3', 'w2b'):
                    for i in range(dict(T0)[k]):
                        wt(k, i)
                for k in ('w1', 'w2a'):
                    assert all((k, i) in waited for i in range(dict(T1)[k]))
        for i in range(max(B1 - WC, 0), B0):
            wt('wob', i)
        assert all((i * 171) >> 9 == i // 3 for i in range(512)) and max(KD, D0) < 512
        assert started == waited, (len(started), len(waited), sorted(started - waited)[:5])
        assert B1 <= 186
        for i in range(B0):
            if B1 + perm('wob', i) >= 186:
                assert i + WC >= UH, i
        assert sorted(perm('wob', i) for i in range(B0)) == list(range(B0))
    simulate()

    @jax.jit
    def kernel_fn(A_x, A_k_cache, A_v_cache, A_wq, A_wo, B_x, B_w1, B_w3, B_w2):
        kT = jnp.swapaxes(A_k_cache, 2, 3).reshape(HD, SK)
        vT = jnp.swapaxes(A_v_cache, 2, 3).reshape(HD, SK)
        return pl.pallas_call(
            _kernel,
            in_specs=[pl.BlockSpec(memory_space=pl.ANY)] * 8,
            out_specs=pl.BlockSpec(memory_space=pltpu.VMEM),
            out_shape=jax.ShapeDtypeStruct((1, 1, D), bf16),
            scratch_shapes=[
                pltpu.VMEM((1, 1, D), bf16),
                pltpu.VMEM((D, HD), bf16),
                pltpu.VMEM((HD, D), bf16),
                pltpu.VMEM((D, F), bf16),
                pltpu.VMEM((D, F), bf16),
                pltpu.VMEM((F, D), bf16),
                pltpu.VMEM((KR, RB, CB), bf16),
                pltpu.VMEM((VR, RB, CB), bf16),
                pltpu.VMEM((2, DH, 128), f32),
                pltpu.VMEM((H, 8, DH), f32),
                pltpu.VMEM((HD, 128), f32),
                pltpu.VMEM((NC * 8, 128), f32),
                pltpu.VMEM((NC, 128), f32),
                pltpu.VMEM((DH, 128), f32),
                pltpu.VMEM((8, D), bf16),
                pltpu.VMEM((8, D), f32),
                pltpu.SemaphoreType.DMA((1,)),
                pltpu.SemaphoreType.DMA((128,)),
                pltpu.SemaphoreType.DMA((1,)),
                pltpu.SemaphoreType.DMA((2,)),
                pltpu.SemaphoreType.DMA((VR,)),
                pltpu.SemaphoreType.DMA((32,)),
            ],
            compiler_params=pltpu.CompilerParams(vmem_limit_bytes=100 * 1024 * 1024,
                                                 disable_bounds_checks=True, disable_semaphore_checks=True),
        )(A_x, kT, vT, A_wq, A_wo, B_w1, B_w3, B_w2)
    return kernel_fn

_impl = make()


@jax.jit
def pallas_recurrent_scan__sliding_block_cached__glu_gated_swiglu__decode_kernel(
        A_x, A_k_cache, A_v_cache, A_wq, A_wo, B_x, B_w1, B_w3, B_w2):
    return _impl(A_x, A_k_cache, A_v_cache, A_wq, A_wo, B_x, B_w1, B_w3, B_w2)
```

```python
import jax
import jax.numpy as jnp
from jax import lax
from jax.experimental import pallas as pl
from jax.experimental.pallas import tpu as pltpu

D, F, H, DH, SK = 640, 1536, 32, 192, 32768
W = min(4096, max(256, SK // 4))
HD = H * DH
NC = W // 128
RB, CB = 64, 256
NRB = DH // RB
NCB = W // CB
UH = NRB * NCB
NKV = H * UH
f32, bf16 = jnp.float32, jnp.bfloat16


def _tree_sum(xs):
    xs = list(xs)
    while len(xs) > 1:
        xs = [xs[i] + xs[i + 1] if i + 1 < len(xs) else xs[i] for i in range(0, len(xs), 2)]
    return xs[0]


def _is_int(i):
    return isinstance(i, int)


def _shr(i, s):
    return i >> s if _is_int(i) else lax.shift_right_logical(i, s)


def _and(i, m):
    return i & m if _is_int(i) else lax.bitwise_and(i, m)


def _mo(i, m):
    return i if _is_int(i) else pl.multiple_of(i, m)


def _compiler_params():
    kw = dict(vmem_limit_bytes=100 * 1024 * 1024, disable_bounds_checks=True)
    try:
        return pltpu.CompilerParams(disable_semaphore_checks=True, **kw)
    except TypeError:
        return pltpu.CompilerParams(**kw)


def _runs(items):
    out, s = [], 0
    for i in range(1, len(items) + 1):
        if i == len(items) or items[i] != items[s]:
            out.append((s, i, items[s]))
            s = i
    return out


def make(KD=48, D0=0, KR=128, VR=128, B1=116, WL=21, PG=4, PG1=4, PG2=2, QP=2):
    NQ, N1, N2, NO = 80, 40, 24, 192
    A = NQ + N1 + N2
    B0 = NO - B1
    T1 = [('wqA', NQ), ('w1', N1), ('w2a', N2), ('K', NKV), ('woa', B1)]
    T0 = [('wqB', NQ), ('w3', N1), ('w2b', N2), ('V', NKV), ('wob', B0)]
    NT = A + NKV + B1
    WLC = WL - D0
    assert KD % 24 == 0 and D0 % 24 == 0 and A % 8 == 0
    QS = A // 8 - 2 * QP
    assert QS * 8 >= NQ

    def locate(lst, t):
        for kind, n in lst:
            if 0 <= t < n:
                return kind, t
            t -= n
        return None, None

    def offset(lst, kind):
        o = 0
        for k, n in lst:
            if k == kind:
                return o
            o += n

    OFF = {k: offset(T1, k) for k, _ in T1}
    OFF.update({k: offset(T0, k) for k, _ in T0})

    CNT = dict(T1 + T0)

    def perm(kind, i):
        pg = {'w1': PG1, 'w3': PG1, 'w2a': PG2, 'w2b': PG2}.get(kind, PG)
        if pg == 1:
            return i
        assert CNT[kind] % pg == 0, (kind, CNT[kind])
        return _and(i, pg - 1) * (CNT[kind] // pg) + _shr(i, pg.bit_length() - 1)

    def _kernel(x_hbm, k_hbm, v_hbm, wq_hbm, wo_hbm, w1_hbm, w3_hbm, w2_hbm, o_ref,
                x_v, wq_v, wo_v, w1_v, w3_v, w2_v, kbuf, vbuf, qbc, qrow, obc, s_scr, p_scr, acc_ref, xn_s, g_s,
                sem_x, sem_1, sem_q, sem_w, sem_v, sem_ob):

        def cp(kind, i):
            s1 = lambda: sem_1.at[_and(i + OFF[kind], 127)]
            if kind in ('wqA', 'wqB'):
                k = _shr(i, 2)
                rt = (0 if kind == 'wqA' else 40) + _and(i, 3) * 10 + _shr(k, 1)
                sl = (pl.ds(_mo(rt * 8, 8), 8), pl.ds(_mo(_and(k, 1) * 3072, 128), 3072))
                sem = s1() if kind == 'wqA' else sem_q.at[0]
                return pltpu.make_async_copy(wq_hbm.at[sl], wq_v.at[sl], sem)
            if kind in ('w1', 'w3'):
                src, dst = (w1_hbm, w1_v) if kind == 'w1' else (w3_hbm, w3_v)
                sl = pl.ds(_mo(perm(kind, i) * 16, 16), 16)
                return pltpu.make_async_copy(src.at[sl], dst.at[sl], s1() if kind == 'w1' else sem_w.at[0])
            if kind in ('w2a', 'w2b'):
                sl = pl.ds(_mo((perm(kind, i) + (0 if kind == 'w2a' else N2)) * 32, 32), 32)
                return pltpu.make_async_copy(w2_hbm.at[sl], w2_v.at[sl], s1() if kind == 'w2a' else sem_w.at[1])
            if kind in ('K', 'V'):
                g, rb = i if isinstance(i, tuple) else divmod(i, NRB)
                n = g * NRB + rb
                src, buf, ring = (k_hbm, kbuf, KR) if kind == 'K' else (v_hbm, vbuf, VR)
                r0 = _mo(_shr(g, 4) * DH + rb * RB, 8)
                c0 = _mo(SK - W + _and(g, NCB - 1) * CB, 128)
                slot = _and(n, ring - 1)
                sem = sem_1.at[_and(n + OFF['K'], 127)] if kind == 'K' else sem_v.at[slot]
                return pltpu.make_async_copy(src.at[pl.ds(r0, RB), pl.ds(c0, CB)], buf.at[slot], sem)
            if kind in ('woa', 'wob'):
                u = perm(kind, i) + (0 if kind == 'woa' else B1)
                sl = pl.ds(_mo(u * 32, 32), 32)
                sem = s1() if kind == 'woa' else sem_ob.at[_and(i, 31)]
                return pltpu.make_async_copy(wo_hbm.at[sl], wo_v.at[sl], sem)
            raise ValueError(kind)

        x_cp = pltpu.make_async_copy(x_hbm, x_v, sem_x.at[0])
        x_cp.start(priority=0)

        def pro(t, c):
            cp('wqA', t).start(priority=1)
            cp('wqB', t).start(priority=0)
            return c
        if D0:
            lax.fori_loop(0, D0, pro, 0)

        def pro1(t, c):
            cp('wqA', t).start(priority=1)
            return c
        assert KD <= NQ
        lax.fori_loop(D0, KD, pro1, 0)

        def layernorm():
            x_cp.wait()
            x = x_v[...].reshape(1, D).astype(f32)
            mu = jnp.mean(x, axis=-1, keepdims=True)
            xc = x - mu
            var = jnp.mean(xc * xc, axis=-1, keepdims=True)
            xn_s[...] = jnp.broadcast_to((xc / jnp.sqrt(var + 1e-5)).astype(bf16), (8, D))

        def q_piece(j):
            c0 = _mo(j * 384, 128)
            q = jnp.dot(xn_s[...], wq_v[:, pl.ds(c0, 384)], preferred_element_type=f32)
            q = q.astype(bf16).astype(f32)
            qrow[2 * j, :, 0:DH] = q[:, 0:DH]
            qrow[2 * j + 1, :, 0:DH] = q[:, DH:2 * DH]

        def build_qbc(h):
            diff = lax.broadcasted_iota(jnp.int32, (8, 128), 1) - lax.broadcasted_iota(jnp.int32, (8, 128), 0)
            slot = _and(h, 1)
            qa = qrow[h, :, 0:128]
            qb_ = qrow[h, :, 128:DH]
            for g in range(DH // 8):
                if g < 16:
                    sel = jnp.where(diff == g * 8, qa, 0.0)
                else:
                    sel = jnp.where(diff[:, 0:64] == (g - 16) * 8, qb_, 0.0)
                col = jnp.sum(sel, axis=1, keepdims=True)
                qbc[slot, pl.ds(g * 8, 8), :] = jnp.broadcast_to(col, (8, 128))

        def qk(n, b, rb, t):
            slot = _and(n, KR - 1)
            qs = _and(b, 1)
            lo, hi = [], []
            for g in range(RB // 16):
                k = kbuf[slot, pl.ds(g * 16, 16), :].astype(f32)
                q = qbc[qs, pl.ds(rb * RB + g * 16, 16), :]
                lo.append(k[:, 0:128] * q)
                hi.append(k[:, 128:256] * q)
            if t is not None:
                lo.append(t[0])
                hi.append(t[1])
            return _tree_sum(lo), _tree_sum(hi)

        def qk_store(t, cb):
            r0 = _mo(cb * 16, 16)
            s_scr[pl.ds(r0, 8), :] = t[0][0:8] + t[0][8:16]
            s_scr[pl.ds(r0 + 8, 8), :] = t[1][0:8] + t[1][8:16]

        def pv(n, cb, rb):
            slot = _and(n, VR - 1)
            p0 = jnp.broadcast_to(p_scr[pl.ds(2 * cb, 1), :], (16, 128))
            p1 = jnp.broadcast_to(p_scr[pl.ds(2 * cb + 1, 1), :], (16, 128))
            for g in range(RB // 16):
                v = vbuf[slot, pl.ds(g * 16, 16), :].astype(f32)
                acc_ref[pl.ds(rb * RB + g * 16, 16), :] += v[:, 0:128] * p0 + v[:, 128:256] * p1

        def softmax():
            rows = [_tree_sum([s_scr[pl.ds(g * 64 + j, 8, stride=8), :] for j in range(8)]) for g in range(NC // 8)]
            s = jnp.concatenate(rows, axis=0) * (DH ** -0.5)
            m = jnp.max(jnp.max(s, axis=0, keepdims=True), axis=1, keepdims=True)
            p = jnp.exp(s - m)
            l = jnp.sum(jnp.sum(p, axis=0, keepdims=True), axis=1, keepdims=True)
            p_scr[...] = p
            return l

        def finalize(h, l):
            o = jnp.sum(acc_ref[...], axis=1, keepdims=True) / l
            obc[pl.ds(_mo(h * DH, 8), DH), :] = jnp.broadcast_to(o, (DH, 128))

        def wo_piece(u, y):
            r0 = _mo(u * 32, 32)
            for g in range(2):
                w = wo_v[pl.ds(r0 + g * 16, 16), :].astype(f32)
                ob = obc[pl.ds(r0 + g * 16, 16), :]
                pr = w * jnp.concatenate([ob] * (D // 128), axis=1)
                y = y + pr[0:8] + pr[8:16]
            return y

        def ffn():
            xn8 = xn_s[...]
            gate = jnp.dot(xn8, w1_v[...], preferred_element_type=f32)
            up = jnp.dot(xn8, w3_v[...], preferred_element_type=f32)
            hh = (gate * jax.nn.sigmoid(gate) * up).astype(bf16)
            ff = jnp.dot(hh, w2_v[...], preferred_element_type=f32)
            g_s[...] = ff * jax.nn.sigmoid(ff)

        def start(kind, i, prio):
            if kind is not None:
                cp(kind, i).start(priority=prio)

        def startA(kind, tt, prio):
            i = tt - OFF[kind]
            if kind in ('K', 'V'):
                gi = lax.shift_right_logical(i * 171, 9)
                cp(kind, (gi, i - gi * NRB)).start(priority=prio)
            else:
                cp(kind, i).start(priority=prio)

        groups = []
        for g in range(A // 8):
            t = g * 8
            groups.append((locate(T1, t)[0], locate(T1, t + KD)[0], locate(T0, t + D0)[0], g >= QS))
        for g0, g1, (kw, k1, k0, has_q) in _runs(groups):
            if g0 == QS:
                layernorm()
                sl = pl.ds(D // 2, D // 2)
                pltpu.make_async_copy(wq_v.at[sl], wq_v.at[sl], sem_q.at[0]).wait()

            def group(g, carry, kw=kw, k1=k1, k0=k0, has_q=has_q):
                for s in range(8):
                    t = g * 8 + s
                    cp(kw, t - OFF[kw]).wait()
                    startA(k1, t + KD, 1)
                    startA(k0, t + D0, 0)
                    if has_q and s % QP == QP - 1:
                        q_piece((g - QS) * (8 // QP) + s // QP)
                return carry

            lax.fori_loop(g0, g1, group, 0)

        def kinds(n):
            return locate(T1, A + n + KD)[0], locate(T0, A + n + D0)[0]

        def iteration(b, cb, do_pv, k1, k0):
            g = b * NCB + cb
            t = None
            for rb in range(NRB):
                n = g * NRB + rb
                cp('K', (g, rb)).wait()
                if do_pv:
                    cp('V', (g - NCB, rb)).wait()
                t = qk(n, b, rb, t)
                if do_pv:
                    pv(n - UH, cb, rb)
                if k1 == 'K':
                    cp('K', (g + KD // NRB, rb)).start(priority=1)
                else:
                    start(k1, A + n + KD - OFF['woa'], 1)
                if k0 == 'V':
                    cp('V', (g + D0 // NRB, rb)).start(priority=0)
                else:
                    start(k0, A + n + D0 - OFF['wob'], 0)
            qk_store(t, cb)

        def block(b, do_pv, segs, l_prev, nxt=True):
            if do_pv:
                acc_ref[...] = jnp.zeros_like(acc_ref)
            for c0, c1, (k1, k0) in segs:
                def body(cb, carry, k1=k1, k0=k0):
                    iteration(b, cb, do_pv, k1, k0)
                    return carry
                lax.fori_loop(c0, c1, body, 0)
            if do_pv:
                finalize(b - 1, l_prev)
            if nxt:
                build_qbc(b + 1)
            return softmax()

        def segs_of(b):
            return _runs([kinds(b * UH + cb * NRB) for cb in range(NCB)])

        plain = [(0, NCB, ('K', 'V'))]
        nplain = max(b for b in range(H) if segs_of(b) == plain) + 1
        build_qbc(0)
        l = block(0, False, plain, None)
        pltpu.make_async_copy(w3_v, w3_v, sem_w.at[0]).wait()
        sl = pl.ds(N2 * 32, N2 * 32)
        pltpu.make_async_copy(w2_v.at[sl], w2_v.at[sl], sem_w.at[1]).wait()
        ffn()
        l = lax.fori_loop(1, nplain, lambda b, l: block(b, True, plain, l), l)
        for b in range(nplain, H):
            l = block(b, True, segs_of(b), l, nxt=b + 1 < H)

        acc_ref[...] = jnp.zeros_like(acc_ref)
        tB = A + NKV
        WC = max(WLC, 0)

        def attrsB(j):
            return (j < UH, locate(T1, tB + j + KD)[0], locate(T0, tB + j + D0)[0], WC <= j < B0 + WC)

        y = jnp.zeros((8, D), f32)
        ticks = [attrsB(j) for j in range(B1)]
        for j0, j1, (do_pv, s1, s0, w0) in _runs(ticks):
            def one(j, y, rb, cb, do_pv=do_pv, s1=s1, s0=s0, w0=w0):
                cp('woa', j).wait()
                if do_pv:
                    cp('V', ((H - 1) * NCB + cb, rb)).wait()
                if w0:
                    cp('wob', j - WC).wait()
                if do_pv:
                    pv((NKV - UH) + cb * NRB + rb, cb, rb)
                y = wo_piece(perm('woa', j), y)
                if w0:
                    y = wo_piece(B1 + perm('wob', j - WC), y)
                start(s1, tB + j + KD - OFF['woa'], 1)
                start(s0, tB + j + D0 - OFF['wob'], 0)
                return y

            if do_pv:
                assert j0 % NRB == 0 and j1 % NRB == 0, (j0, j1)

                def body3(cb, y, one=one):
                    for rb in range(NRB):
                        y = one(cb * NRB + rb, y, rb, cb)
                    return y
                y = lax.fori_loop(j0 // NRB, j1 // NRB, body3, y)
            else:
                y = lax.fori_loop(j0, j1, lambda j, y, one=one: one(j, y, None, None), y)
            if j1 == UH:
                finalize(H - 1, l)

        if B1 - WC < B0:
            def tail(i, y):
                cp('wob', i).wait()
                return wo_piece(B1 + perm('wob', i), y)
            y = lax.fori_loop(B1 - WC, B0, tail, y)

        s = jnp.sum(y, axis=0, keepdims=True)
        out = x_v[...].reshape(1, D).astype(f32) + s * g_s[0:1]
        o_ref[...] = out.astype(bf16).reshape(1, 1, D)

    def simulate():
        started, waited = set(), set()
        WC = max(WLC, 0)
        def st(k, i):
            n = dict(T1 + T0)[k]
            assert 0 <= i < n, (k, i)
            assert (k, i) not in started
            started.add((k, i))
            if k in OFF and k in dict(T1):
                gi = i + OFF[k] - 128
                if gi >= 0:
                    assert locate(T1, gi) in waited, (k, i)
            if k == 'K' and i >= KR:
                assert ('K', i - KR) in waited
            if k == 'V' and i >= VR:
                assert ('V', i - VR) in waited
            if k == 'wob' and i >= 32:
                assert ('wob', i - 32) in waited
        def wt(k, i):
            assert (k, i) in started, ('wait before start', k, i)
            assert (k, i) not in waited
            waited.add((k, i))
        for t in range(D0):
            st(*locate(T0, t))
        for t in range(KD):
            st(*locate(T1, t))
        for t in range(NT):
            k, i = locate(T1, t)
            wt(k, i)
            if k == 'K' and i >= UH:
                wt('V', i - UH)
            if k == 'woa':
                if i < UH:
                    wt('V', NKV - UH + i)
                if WC <= i < B0 + WC:
                    wt('wob', i - WC)
            k1, i1 = locate(T1, t + KD)
            if k1 is not None:
                st(k1, i1)
            k0, i0 = locate(T0, t + D0)
            if k0 is not None:
                st(k0, i0)
            if t == QS * 8 - 1:
                for u in range(NQ):
                    assert ('wqA', u) in waited
                    wt('wqB', u)
            if t == A + UH - 1:
                for k in ('w3', 'w2b'):
                    for i in range(dict(T0)[k]):
                        wt(k, i)
                for k in ('w1', 'w2a'):
                    assert all((k, i) in waited for i in range(dict(T1)[k]))
        for i in range(max(B1 - WC, 0), B0):
            wt('wob', i)
        assert all((i * 171) >> 9 == i // 3 for i in range(512)) and max(KD, D0) < 512
        assert started == waited, (len(started), len(waited), sorted(started - waited)[:5])
        assert B1 <= 186
        for i in range(B0):
            if B1 + perm('wob', i) >= 186:
                assert i + WC >= UH, i
        assert sorted(perm('wob', i) for i in range(B0)) == list(range(B0))
    simulate()

    @jax.jit
    def kernel_fn(A_x, A_k_cache, A_v_cache, A_wq, A_wo, B_x, B_w1, B_w3, B_w2):
        kT = jnp.swapaxes(A_k_cache, 2, 3).reshape(HD, SK)
        vT = jnp.swapaxes(A_v_cache, 2, 3).reshape(HD, SK)
        return pl.pallas_call(
            _kernel,
            in_specs=[pl.BlockSpec(memory_space=pl.ANY)] * 8,
            out_specs=pl.BlockSpec(memory_space=pltpu.VMEM),
            out_shape=jax.ShapeDtypeStruct((1, 1, D), bf16),
            scratch_shapes=[
                pltpu.VMEM((1, 1, D), bf16),
                pltpu.VMEM((D, HD), bf16),
                pltpu.VMEM((HD, D), bf16),
                pltpu.VMEM((D, F), bf16),
                pltpu.VMEM((D, F), bf16),
                pltpu.VMEM((F, D), bf16),
                pltpu.VMEM((KR, RB, CB), bf16),
                pltpu.VMEM((VR, RB, CB), bf16),
                pltpu.VMEM((2, DH, 128), f32),
                pltpu.VMEM((H, 8, DH), f32),
                pltpu.VMEM((HD, 128), f32),
                pltpu.VMEM((NC * 8, 128), f32),
                pltpu.VMEM((NC, 128), f32),
                pltpu.VMEM((DH, 128), f32),
                pltpu.VMEM((8, D), bf16),
                pltpu.VMEM((8, D), f32),
                pltpu.SemaphoreType.DMA((1,)),
                pltpu.SemaphoreType.DMA((128,)),
                pltpu.SemaphoreType.DMA((1,)),
                pltpu.SemaphoreType.DMA((2,)),
                pltpu.SemaphoreType.DMA((VR,)),
                pltpu.SemaphoreType.DMA((32,)),
            ],
            compiler_params=_compiler_params(),
        )(A_x, kT, vT, A_wq, A_wo, B_w1, B_w3, B_w2)
    return kernel_fn

_impl = make()


@jax.jit
def pallas_recurrent_scan__sliding_block_cached__glu_gated_swiglu__decode_kernel(
        A_x, A_k_cache, A_v_cache, A_wq, A_wo, B_x, B_w1, B_w3, B_w2):
    return _impl(A_x, A_k_cache, A_v_cache, A_wq, A_wo, B_x, B_w1, B_w3, B_w2)
```
